```python
import os as _os
_os.environ.setdefault("JAX_PLATFORMS", "cpu")
import jax
import jax.numpy as jnp

def _softmax(x, axis=-1):
    return jax.nn.softmax(x, axis=axis)
def _gelu(x):
    return jax.nn.gelu(x, approximate=True)
def _silu(x):
    return jax.nn.silu(x)
def _sigmoid(x):
    return jax.nn.sigmoid(x)
def _layernorm(x, axis=-1, eps=1e-5):
    m = jnp.mean(x, axis=axis, keepdims=True)
    v = jnp.var(x, axis=axis, keepdims=True)
    return (x - m) / jnp.sqrt(v + eps)
def _scatter_add(tgt, idx, src, axis=0):
    return tgt.at[idx].add(src)
def _segment_sum(src, seg, n):
    return jax.ops.segment_sum(src, seg, n)
class _Rng:
    def __init__(self, key):
        self._k = key
    def _next(self):
        self._k, sub = jax.random.split(self._k)
        return sub
    def normal(self, shape):
        return jax.random.normal(self._next(), shape, dtype=jnp.bfloat16)
    def randint(self, lo, hi, shape):
        return jax.random.randint(self._next(), shape, lo, hi, dtype=jnp.int32)
    def uniform(self, shape, lo=0.0, hi=1.0):
        return jax.random.uniform(self._next(), shape, jnp.bfloat16, lo, hi)
    def permutation(self, n):
        return jax.random.permutation(self._next(), n)


kernel_name = 'standalone__mha_softmax__near_ridge'

def setup_inputs():
    _rng = _Rng(jax.random.key(int.from_bytes(__import__("os").urandom(4), "little")))
    _w = (lambda a: (lambda t: t.astype(jnp.bfloat16) if jnp.issubdtype(t.dtype, jnp.floating) else t)(jnp.asarray(a)))
    B, H, Sq, Sk, D = 8, 32, 384, 512, 128
    return {
        "q": _w((lambda *s: _rng.normal(s) * 0.4)(B, H, Sq, D)),
        "k": _w((lambda *s: _rng.normal(s) * 0.4)(B, H, Sk, D)),
        "v": _w((lambda *s: _rng.normal(s) * 0.05)(B, H, Sk, D)),
    }

def reference(q, k, v):
    scale = q.shape[-1] ** -0.5
    scores = jnp.einsum("bhqd,bhkd->bhqk", q, k) * scale
    p = _softmax(scores, axis=-1)
    return jnp.einsum("bhqk,bhkd->bhqd", p, v)
```

```python
import jax
import jax.numpy as jnp
from jax import lax
from jax.experimental import pallas as pl
from jax.experimental.pallas import tpu as pltpu

LOG2E = 1.4426950408889634

REGIONS = 4
GROUP = 8
READ_STEPS_PER_HEAD = 16
READ_STEPS_PER_ITER = 39
WRITES_PER_HEAD = 2
WRITES_PER_ITER = 16
FIRST_WRITES = 4
MIN_FIRST_READS = 45


def _attend(q, k, v):
    scale = q.shape[-1] ** -0.5 * LOG2E
    s = lax.dot_general(
        q, k, (((1,), (1,)), ((), ())), preferred_element_type=jnp.float32
    )
    m = jnp.max(s, axis=-1, keepdims=True)
    p = jnp.exp2((s - m) * scale)
    l = jnp.sum(p, axis=-1, keepdims=True)
    o = jnp.dot(p.astype(v.dtype), v, preferred_element_type=jnp.float32)
    r = pl.reciprocal(l, approx=True)
    r = r * (2.0 - l * r)
    return (o * r).astype(q.dtype)


def _spread(n, parts):
    return [(n * (i + 1)) // parts - (n * i) // parts for i in range(parts)]


@jax.jit
def pallas_standalone__mha_softmax__near_ridge_kernel(
    q: jax.Array,
    k: jax.Array,
    v: jax.Array,
):
    batch, heads, sq, d = q.shape
    sk = k.shape[2]
    n_heads = batch * heads
    region_heads = n_heads // REGIONS
    group_rows = GROUP // REGIONS
    n_groups = n_heads // GROUP

    q_rows, k_rows = sq // READ_STEPS_PER_HEAD, sk // READ_STEPS_PER_HEAD
    o_rows = sq // WRITES_PER_HEAD
    n_reads = region_heads * READ_STEPS_PER_HEAD
    group_reads = group_rows * READ_STEPS_PER_HEAD
    n_writes = region_heads * WRITES_PER_HEAD
    group_writes = group_rows * WRITES_PER_HEAD

    read_iters = (n_reads - MIN_FIRST_READS) // READ_STEPS_PER_ITER
    first_reads = n_reads - read_iters * READ_STEPS_PER_ITER
    write_iters = n_groups - read_iters
    last_write = FIRST_WRITES + write_iters * WRITES_PER_ITER
    assert group_reads & (group_reads - 1) == 0
    assert all(
        min(n_reads, first_reads + READ_STEPS_PER_ITER * g) >= group_reads * (g + 1)
        for g in range(n_groups)
    )
    assert all(
        FIRST_WRITES + WRITES_PER_ITER * (i + 1) <= group_writes * (read_iters + i)
        for i in range(write_iters)
    )
    assert last_write <= n_writes

    def rows(start, size):
        if not isinstance(start, int):
            start = pl.multiple_of(start, 8)
        return pl.ds(start, size)

    def kernel(q_hbm, k_hbm, v_hbm, o_hbm, q_buf, k_buf, v_buf, o_buf, r_sem, w_sem):
        def reads(step, count, group):
            copies = []
            for hbm, buf, size in (
                (q_hbm, q_buf, q_rows),
                (k_hbm, k_buf, k_rows),
                (v_hbm, v_buf, k_rows),
            ):
                sl = rows(step * size, count * size)
                copies.append(
                    pltpu.make_async_copy(hbm.at[:, sl], buf.at[:, sl], r_sem.at[group])
                )
            return copies

        def start_read(step):
            group = step >> (group_reads.bit_length() - 1)
            for copy, priority in zip(reads(step, 1, group), (0, 1, 1)):
                copy.start(priority=priority)

        def writes(step, count):
            sl = rows(step * o_rows, count * o_rows)
            return pltpu.make_async_copy(o_buf.at[:, sl], o_hbm.at[:, sl], w_sem)

        def start_write(step):
            writes(step, 1).start(priority=1)

        def run_group(group, start, first, count):
            for copy in reads(group * group_reads, group_reads, group):
                copy.wait()
            done = 0
            for u, n in enumerate(_spread(count, GROUP)):
                for i in range(done, done + n):
                    start(first + i)
                done += n
                region, head = u % REGIONS, group * group_rows + u // REGIONS
                q_sl = pl.ds(pl.multiple_of(head * sq, sq), sq)
                k_sl = pl.ds(pl.multiple_of(head * sk, sk), sk)
                o_buf[region, q_sl] = _attend(
                    q_buf[region, q_sl], k_buf[region, k_sl], v_buf[region, k_sl]
                )

        for step in range(first_reads):
            start_read(step)

        @pl.loop(0, read_iters)
        def _(i):
            first = first_reads + i * READ_STEPS_PER_ITER
            run_group(i, start_read, first, READ_STEPS_PER_ITER)

        for step in range(FIRST_WRITES):
            start_write(step)

        @pl.loop(0, write_iters)
        def _(i):
            first = FIRST_WRITES + i * WRITES_PER_ITER
            run_group(read_iters + i, start_write, first, WRITES_PER_ITER)

        for step in range(last_write, n_writes):
            start_write(step)
        writes(0, n_writes).wait()

    q_shape = (REGIONS, region_heads * sq, d)
    k_shape = (REGIONS, region_heads * sk, d)
    out = pl.pallas_call(
        kernel,
        in_specs=[pl.BlockSpec(memory_space=pl.ANY)] * 3,
        out_specs=pl.BlockSpec(memory_space=pl.ANY),
        out_shape=jax.ShapeDtypeStruct(q_shape, q.dtype),
        scratch_shapes=[
            pltpu.VMEM(q_shape, q.dtype),
            pltpu.VMEM(k_shape, k.dtype),
            pltpu.VMEM(k_shape, v.dtype),
            pltpu.VMEM(q_shape, q.dtype),
            pltpu.SemaphoreType.DMA((n_groups,)),
            pltpu.SemaphoreType.DMA(()),
        ],
        compiler_params=pltpu.CompilerParams(
            vmem_limit_bytes=126 * 1024 * 1024, disable_bounds_checks=True
        ),
    )(q.reshape(q_shape), k.reshape(k_shape), v.reshape(k_shape))
    return out.reshape(q.shape)
```

```python
import jax
import jax.numpy as jnp
from jax import lax
from jax.experimental import pallas as pl
from jax.experimental.pallas import tpu as pltpu

LOG2E = 1.4426950408889634

GROUP = 8
PIECES = 4
READ_ITERS = 25
READS_PER_ITER = 38
FIRST_WRITES = 26
WRITES_PER_ITER = 14


def _attend(q, k, v):
    scale = q.shape[-1] ** -0.5 * LOG2E
    s = lax.dot_general(
        q, k, (((1,), (1,)), ((), ())), preferred_element_type=jnp.float32
    )
    m = jnp.max(s, axis=-1, keepdims=True)
    p = jnp.exp2((s - m) * scale)
    l = jnp.sum(p, axis=-1, keepdims=True)
    o = jnp.dot(p.astype(v.dtype), v, preferred_element_type=jnp.float32)
    r = pl.reciprocal(l, approx=True)
    r = r * (2.0 - l * r)
    return (o * r).astype(q.dtype)


def _spread(n, parts):
    return [(n * (i + 1)) // parts - (n * i) // parts for i in range(parts)]


def _slice(start, size, multiple):
    if not isinstance(start, int):
        start = pl.multiple_of(start, multiple)
    return pl.ds(start, size)


@jax.jit
def pallas_standalone__mha_softmax__near_ridge_kernel(
    q: jax.Array,
    k: jax.Array,
    v: jax.Array,
):
    batch, heads, sq, d = q.shape
    sk = k.shape[2]
    n_groups = batch * heads // GROUP

    group_reads = GROUP * PIECES
    n_reads = n_groups * group_reads
    first_reads = n_reads - READ_ITERS * READS_PER_ITER
    write_iters = n_groups - READ_ITERS
    n_writes = n_groups * PIECES
    last_write = FIRST_WRITES + write_iters * WRITES_PER_ITER
    assert all(
        min(n_reads, first_reads + READS_PER_ITER * g) >= group_reads * (g + 1)
        for g in range(n_groups)
    )
    assert all(
        FIRST_WRITES + WRITES_PER_ITER * (i + 1) <= PIECES * (READ_ITERS + i)
        for i in range(write_iters)
    )
    assert last_write <= n_writes
    region_bits, group_bits = GROUP.bit_length() - 1, group_reads.bit_length() - 1
    assert GROUP == 1 << region_bits and group_reads == 1 << group_bits

    def kernel(q_hbm, k_hbm, v_hbm, o_hbm, q_buf, k_buf, v_buf, o_buf, write_sem):
        inputs = ((q_hbm, q_buf, sq, 0), (k_hbm, k_buf, sk, 1), (v_hbm, v_buf, sk, 1))

        def start_write(step):
            rows = sq // PIECES
            sl = _slice(step * rows, rows, 8)
            copy = pltpu.make_async_copy(o_buf.at[:, sl], o_hbm.at[:, sl], write_sem)
            copy.start(priority=1)

        def run(read_sems):
            def start_read(step):
                region, piece = step & (GROUP - 1), step >> region_bits
                sem = read_sems.at[step >> group_bits]
                for hbm, buf, seq, priority in inputs:
                    rows = seq // PIECES
                    at = (pl.ds(region, 1), _slice(piece * rows, rows, 8))
                    copy = pltpu.make_async_copy(hbm.at[at], buf.at[at], sem)
                    copy.start(priority=priority)

            def run_group(g, start, first, count):
                for hbm, buf, seq, _ in inputs:
                    sl = _slice(g * seq, seq, seq)
                    pltpu.make_async_copy(
                        hbm.at[:, sl], buf.at[:, sl], read_sems.at[g]
                    ).wait()
                q_rows, k_rows = _slice(g * sq, sq, sq), _slice(g * sk, sk, sk)
                for region, n in enumerate(_spread(count, GROUP)):
                    for i in range(n):
                        start(first + i)
                    first += n
                    o_buf[region, q_rows] = _attend(
                        q_buf[region, q_rows],
                        k_buf[region, k_rows],
                        v_buf[region, k_rows],
                    )

            for step in range(first_reads):
                start_read(step)

            @pl.loop(0, READ_ITERS)
            def _(i):
                first = first_reads + i * READS_PER_ITER
                run_group(i, start_read, first, READS_PER_ITER)

            for step in range(FIRST_WRITES):
                start_write(step)

            @pl.loop(0, write_iters)
            def _(i):
                first = FIRST_WRITES + i * WRITES_PER_ITER
                run_group(READ_ITERS + i, start_write, first, WRITES_PER_ITER)

            for step in range(last_write, n_writes):
                start_write(step)

        pl.run_scoped(run, pltpu.SemaphoreType.DMA((n_groups,)))
        pltpu.make_async_copy(o_buf, o_hbm, write_sem).wait()

    q_shape = (GROUP, n_groups * sq, d)
    k_shape = (GROUP, n_groups * sk, d)
    out = pl.pallas_call(
        kernel,
        in_specs=[pl.BlockSpec(memory_space=pl.ANY)] * 3,
        out_specs=pl.BlockSpec(memory_space=pl.ANY),
        out_shape=jax.ShapeDtypeStruct(q_shape, q.dtype),
        scratch_shapes=[
            pltpu.VMEM(q_shape, q.dtype),
            pltpu.VMEM(k_shape, k.dtype),
            pltpu.VMEM(k_shape, v.dtype),
            pltpu.VMEM(q_shape, q.dtype),
            pltpu.SemaphoreType.DMA(()),
        ],
        compiler_params=pltpu.CompilerParams(vmem_limit_bytes=124 * 1024 * 1024),
    )(q.reshape(q_shape), k.reshape(k_shape), v.reshape(k_shape))
    return out.reshape(q.shape)
```

```python
import jax
import jax.numpy as jnp
from jax import lax
from jax.experimental import pallas as pl
from jax.experimental.pallas import tpu as pltpu

LOG2E = 1.4426950408889634

GROUP = 8
PIECES = 4
READ_ITERS = 25
READS_PER_ITER = 38
FIRST_WRITES = 26
WRITES_PER_ITER = 14


def _attend(q, k, v):
    scale = q.shape[-1] ** -0.5 * LOG2E
    s = lax.dot_general(
        q, k, (((1,), (1,)), ((), ())), preferred_element_type=jnp.float32
    )
    m = jnp.max(s, axis=-1, keepdims=True)
    p = jnp.exp2((s - m) * scale)
    l = jnp.sum(p, axis=-1, keepdims=True)
    o = jnp.dot(p.astype(v.dtype), v, preferred_element_type=jnp.float32)
    r = pl.reciprocal(l, approx=True)
    r = r * (2.0 - l * r)
    return (o * r).astype(q.dtype)


def _spread(n, parts):
    return [(n * (i + 1)) // parts - (n * i) // parts for i in range(parts)]


def _slice(start, size, multiple):
    if not isinstance(start, int):
        start = pl.multiple_of(start, multiple)
    return pl.ds(start, size)


@jax.jit
def pallas_standalone__mha_softmax__near_ridge_kernel(
    q: jax.Array,
    k: jax.Array,
    v: jax.Array,
):
    batch, heads, sq, d = q.shape
    sk = k.shape[2]
    n_groups = batch * heads // GROUP

    group_reads = GROUP * PIECES
    n_reads = n_groups * group_reads
    first_reads = n_reads - READ_ITERS * READS_PER_ITER
    write_iters = n_groups - READ_ITERS
    n_writes = n_groups * PIECES
    last_write = FIRST_WRITES + write_iters * WRITES_PER_ITER
    assert all(
        min(n_reads, first_reads + READS_PER_ITER * g) >= group_reads * (g + 1)
        for g in range(n_groups)
    )
    assert all(
        FIRST_WRITES + WRITES_PER_ITER * (i + 1) <= PIECES * (READ_ITERS + i)
        for i in range(write_iters)
    )
    assert last_write <= n_writes
    region_bits, group_bits = GROUP.bit_length() - 1, group_reads.bit_length() - 1
    assert GROUP == 1 << region_bits and group_reads == 1 << group_bits

    def kernel(q_hbm, k_hbm, v_hbm, o_hbm, q_buf, k_buf, v_buf, o_buf):
        def run(q_sems, k_sems, v_sems, o_sem):
            inputs = (
                (q_hbm, q_buf, q_sems, sq, 0),
                (k_hbm, k_buf, k_sems, sk, 1),
                (v_hbm, v_buf, v_sems, sk, 1),
            )

            def start_read(step):
                region, piece = step & (GROUP - 1), step >> region_bits
                for hbm, buf, sems, seq, priority in inputs:
                    rows = seq // PIECES
                    at = (pl.ds(region, 1), _slice(piece * rows, rows, 8))
                    pltpu.make_async_copy(
                        hbm.at[at], buf.at[at], sems.at[step >> group_bits]
                    ).start(priority=priority)

            def start_write(step):
                rows = sq // PIECES
                sl = _slice(step * rows, rows, 8)
                pltpu.make_async_copy(o_buf.at[:, sl], o_hbm.at[:, sl], o_sem).start(
                    priority=1
                )

            def run_group(g, start, first, count):
                for hbm, buf, sems, seq, _ in inputs:
                    sl = _slice(g * seq, seq, seq)
                    pltpu.make_async_copy(
                        hbm.at[:, sl], buf.at[:, sl], sems.at[g]
                    ).wait()
                q_rows, k_rows = _slice(g * sq, sq, sq), _slice(g * sk, sk, sk)
                for region, n in enumerate(_spread(count, GROUP)):
                    for i in range(n):
                        start(first + i)
                    first += n
                    o_buf[region, q_rows] = _attend(
                        q_buf[region, q_rows],
                        k_buf[region, k_rows],
                        v_buf[region, k_rows],
                    )

            for step in range(first_reads):
                start_read(step)

            @pl.loop(0, READ_ITERS)
            def _(i):
                first = first_reads + i * READS_PER_ITER
                run_group(i, start_read, first, READS_PER_ITER)

            for step in range(FIRST_WRITES):
                start_write(step)

            @pl.loop(0, write_iters)
            def _(i):
                first = FIRST_WRITES + i * WRITES_PER_ITER
                run_group(READ_ITERS + i, start_write, first, WRITES_PER_ITER)

            for step in range(last_write, n_writes):
                start_write(step)
            pltpu.make_async_copy(o_buf, o_hbm, o_sem).wait()

        group_sems = pltpu.SemaphoreType.DMA((n_groups,))
        pl.run_scoped(
            run, group_sems, group_sems, group_sems, pltpu.SemaphoreType.DMA(())
        )

    q_shape = (GROUP, n_groups * sq, d)
    k_shape = (GROUP, n_groups * sk, d)
    out = pl.pallas_call(
        kernel,
        in_specs=[pl.BlockSpec(memory_space=pl.ANY)] * 3,
        out_specs=pl.BlockSpec(memory_space=pl.ANY),
        out_shape=jax.ShapeDtypeStruct(q_shape, q.dtype),
        scratch_shapes=[
            pltpu.VMEM(q_shape, q.dtype),
            pltpu.VMEM(k_shape, k.dtype),
            pltpu.VMEM(k_shape, v.dtype),
            pltpu.VMEM(q_shape, q.dtype),
        ],
        compiler_params=pltpu.CompilerParams(vmem_limit_bytes=124 * 1024 * 1024),
    )(q.reshape(q_shape), k.reshape(k_shape), v.reshape(k_shape))
    return out.reshape(q.shape)
```

```python
import jax
import jax.numpy as jnp
from jax import lax
from jax.experimental import pallas as pl
from jax.experimental.pallas import tpu as pltpu

LOG2E = 1.4426950408889634

GROUP = 8
PIECES = 4
READ_ITERS = 25
READS_PER_ITER = 38
FIRST_WRITES = 26
WRITES_PER_ITER = 14


def _attend(q, k, v):
    scale = q.shape[-1] ** -0.5 * LOG2E
    s = lax.dot_general(
        q, k, (((1,), (1,)), ((), ())), preferred_element_type=jnp.float32
    )
    m = jnp.max(s, axis=-1, keepdims=True)
    p = jnp.exp2((s - m) * scale)
    l = jnp.sum(p, axis=-1, keepdims=True)
    o = jnp.dot(p.astype(v.dtype), v, preferred_element_type=jnp.float32)
    r = pl.reciprocal(l, approx=True)
    r = r * (2.0 - l * r)
    return (o * r).astype(q.dtype)


def _spread(n, parts):
    return [(n * (i + 1)) // parts - (n * i) // parts for i in range(parts)]


def _slice(start, size):
    if not isinstance(start, int):
        start = pl.multiple_of(start, 16)
    return pl.ds(start, size)


@jax.jit
def pallas_standalone__mha_softmax__near_ridge_kernel(
    q: jax.Array,
    k: jax.Array,
    v: jax.Array,
):
    batch, heads, sq, d = q.shape
    sk = k.shape[2]
    n_groups = batch * heads // GROUP

    group_reads = GROUP * PIECES
    n_reads = n_groups * group_reads
    first_reads = n_reads - READ_ITERS * READS_PER_ITER
    write_iters = n_groups - READ_ITERS
    n_writes = n_groups * PIECES
    last_write = FIRST_WRITES + write_iters * WRITES_PER_ITER
    assert all(
        min(n_reads, first_reads + READS_PER_ITER * g) >= group_reads * (g + 1)
        for g in range(n_groups)
    )
    assert all(
        FIRST_WRITES + WRITES_PER_ITER * (i + 1) <= PIECES * (READ_ITERS + i)
        for i in range(write_iters)
    )
    assert last_write <= n_writes
    region_bits, group_bits = GROUP.bit_length() - 1, group_reads.bit_length() - 1
    assert GROUP == 1 << region_bits and group_reads == 1 << group_bits

    q_rows, k_rows = sq // PIECES, sk // PIECES

    def kernel(q_hbm, k_hbm, v_hbm, o_hbm, in_buf, out_buf):
        inputs = (
            (q_hbm, 0, q_rows, 0),
            (k_hbm, q_rows, k_rows, 1),
            (v_hbm, q_rows + k_rows, k_rows, 1),
        )

        def run(read_sems, write_sem):
            def start_read(step):
                region, piece = step & (GROUP - 1), step >> region_bits
                for hbm, offset, rows, priority in inputs:
                    pltpu.make_async_copy(
                        hbm.at[region, _slice(piece * rows, rows)],
                        in_buf.at[step, pl.ds(offset, rows)],
                        read_sems.at[step >> group_bits],
                    ).start(priority=priority)

            def start_write(step):
                rows = _slice(step * q_rows, q_rows)
                pltpu.make_async_copy(
                    out_buf.at[:, rows], o_hbm.at[:, rows], write_sem
                ).start(priority=1)

            def run_group(g, start, first, count):
                group = in_buf.at[pl.ds(g * group_reads, group_reads)]
                pltpu.make_async_copy(group, group, read_sems.at[g]).wait()
                for region, n in enumerate(_spread(count, GROUP)):
                    for i in range(n):
                        start(first + i)
                    first += n
                    q_head, k_head, v_head = (
                        jnp.concatenate(
                            [
                                group[piece * GROUP + region, pl.ds(offset, rows)]
                                for piece in range(PIECES)
                            ]
                        )
                        for _, offset, rows, _ in inputs
                    )
                    out_buf[region, _slice(g * sq, sq)] = _attend(
                        q_head, k_head, v_head
                    )

            for step in range(first_reads):
                start_read(step)

            @pl.loop(0, READ_ITERS)
            def _(i):
                first = first_reads + i * READS_PER_ITER
                run_group(i, start_read, first, READS_PER_ITER)

            for step in range(FIRST_WRITES):
                start_write(step)

            @pl.loop(0, write_iters)
            def _(i):
                first = FIRST_WRITES + i * WRITES_PER_ITER
                run_group(READ_ITERS + i, start_write, first, WRITES_PER_ITER)

            for step in range(last_write, n_writes):
                start_write(step)
            pltpu.make_async_copy(out_buf, o_hbm, write_sem).wait()

        pl.run_scoped(
            run, pltpu.SemaphoreType.DMA((n_groups,)), pltpu.SemaphoreType.DMA(())
        )

    q_shape = (GROUP, n_groups * sq, d)
    k_shape = (GROUP, n_groups * sk, d)
    out = pl.pallas_call(
        kernel,
        in_specs=[pl.BlockSpec(memory_space=pl.ANY)] * 3,
        out_specs=pl.BlockSpec(memory_space=pl.ANY),
        out_shape=jax.ShapeDtypeStruct(q_shape, q.dtype),
        scratch_shapes=[
            pltpu.VMEM((n_reads, q_rows + 2 * k_rows, d), q.dtype),
            pltpu.VMEM(q_shape, q.dtype),
        ],
        compiler_params=pltpu.CompilerParams(vmem_limit_bytes=124 * 1024 * 1024),
    )(q.reshape(q_shape), k.reshape(k_shape), v.reshape(k_shape))
    return out.reshape(q.shape)
```
